```python
import jax
import jax.numpy as jnp

def _softmax(x, axis=-1):
    return jax.nn.softmax(x, axis=axis)
def _gelu(x):
    return jax.nn.gelu(x, approximate=True)
def _silu(x):
    return jax.nn.silu(x)
def _sigmoid(x):
    return jax.nn.sigmoid(x)
def _layernorm(x, axis=-1, eps=1e-5):
    m = jnp.mean(x, axis=axis, keepdims=True)
    v = jnp.var(x, axis=axis, keepdims=True)
    return (x - m) / jnp.sqrt(v + eps)
def _scatter_add(tgt, idx, src, axis=0):
    return tgt.at[idx].add(src)
def _segment_sum(src, seg, n):
    return jax.ops.segment_sum(src, seg, n)
class _Rng:
    def __init__(self, key):
        self._k = key
    def _next(self):
        self._k, sub = jax.random.split(self._k)
        return sub
    def normal(self, shape):
        return jax.random.normal(self._next(), shape, dtype=jnp.bfloat16)
    def randint(self, lo, hi, shape):
        return jax.random.randint(self._next(), shape, lo, hi, dtype=jnp.int32)
    def uniform(self, shape, lo=0.0, hi=1.0):
        return jax.random.uniform(self._next(), shape, jnp.bfloat16, lo, hi)
    def permutation(self, n):
        return jax.random.permutation(self._next(), n)


kernel_name = 'parallel_sum__compressed_kv_cla__geglu_ffn__decode'

def _fwd_setup_inputs():
    _rng = _Rng(jax.random.key(int.from_bytes(__import__("os").urandom(4), "little")))
    _w = (lambda a: (lambda t: t.astype(jnp.bfloat16) if jnp.issubdtype(t.dtype, jnp.floating) else t)(jnp.asarray(a)))
    def _A_setup():
        B, H, Sq, Sk, D, M = 8, 32, 1, 4096, 128, 512
        Dc = 4 * D
        return {
            "x": _w((lambda *s: _rng.normal(s) * 0.05)(B, Sq, M)),
            "c_kv": _w((lambda *s: _rng.normal(s) * 0.05)(B, Sk, Dc)),
            "w_q": _w((lambda *s: _rng.normal(s) * 0.05)(M, H, D) * (M ** -0.5)),
            "w_uk": _w((lambda *s: _rng.normal(s) * 0.05)(Dc, H, D) * (Dc ** -0.5)),
            "w_uv": _w((lambda *s: _rng.normal(s) * 0.05)(Dc, H, D) * (Dc ** -0.5)),
            "w_o": _w((lambda *s: _rng.normal(s) * 0.05)(H, D, M) * ((H * D) ** -0.5)),
        }
    _A_in = _A_setup()

    def _B_setup():
        B, S, D, F = 8, 1, 512, 1376
        return {
            "x": _w((lambda *s: _rng.normal(s) * 0.05)(B, S, D)),
            "w_gate": _w((lambda *s: _rng.normal(s) * 0.05)(D, F)),
            "w_up": _w((lambda *s: _rng.normal(s) * 0.05)(D, F)),
            "w_down": _w((lambda *s: _rng.normal(s) * 0.05)(F, D)),
        }
    _B_in = _B_setup()

    return {
        "A_x": _A_in["x"],
        "A_c_kv": _A_in["c_kv"],
        "A_w_q": _A_in["w_q"],
        "A_w_uk": _A_in["w_uk"],
        "A_w_uv": _A_in["w_uv"],
        "A_w_o": _A_in["w_o"],
        "B_x": _B_in["x"],
        "B_w_gate": _B_in["w_gate"],
        "B_w_up": _B_in["w_up"],
        "B_w_down": _B_in["w_down"],
    }

def _fwd_reference(A_x, A_c_kv, A_w_q, A_w_uk, A_w_uv, A_w_o, B_x, B_w_gate, B_w_up, B_w_down):
    def _A_ref(x, c_kv, w_q, w_uk, w_uv, w_o):
        B, Sq, M = x.shape[0], x.shape[1], x.shape[2]
        Sk = c_kv.shape[1]
        H, D = w_q.shape[1], w_q.shape[2]
        q = jnp.einsum("bqm,mhd->bhqd", x, w_q)
        k = jnp.einsum("bkc,chd->bhkd", c_kv, w_uk)
        v = jnp.einsum("bkc,chd->bhkd", c_kv, w_uv)
        scores = jnp.einsum("bhqd,bhkd->bhqk", q, k) * (D ** -0.5)
        off = Sk - Sq
        qi = jnp.arange(Sq)[:, None]
        kj = jnp.arange(Sk)[None, :]
        cmask = kj <= (qi + off)
        scores = jnp.where(cmask[None, None], scores, -1e9)
        p = _softmax(scores, axis=-1)
        ctx = jnp.einsum("bhqk,bhkd->bhqd", p, v)
        return jnp.einsum("bhqd,hdm->bqm", ctx, w_o)

    def _B_ref(x, w_gate, w_up, w_down):
        return (_gelu(x @ w_gate) * (x @ w_up)) @ w_down

    x = A_x
    xn = _layernorm(x, axis=-1)
    return x + _A_ref(xn, A_c_kv, A_w_q, A_w_uk, A_w_uv, A_w_o) + _B_ref(xn, B_w_gate, B_w_up, B_w_down)


def setup_inputs():
    _inp = _fwd_setup_inputs()
    _gk = jax.random.fold_in(jax.random.key(int.from_bytes(__import__("os").urandom(4), "little")), 2**31 - 1)
    _shapes = [[8, 1, 512]]
    _dtypes = ['bfloat16']
    _gks = jax.random.split(_gk, len(_shapes))
    _gs = [jax.random.normal(k, s, dtype=jnp.dtype(d)) * 0.05 for k, s, d in zip(_gks, _shapes, _dtypes)]
    _inp["grad_out"] = _gs[0]
    return _inp

def reference(A_x, A_c_kv, A_w_q, A_w_uk, A_w_uv, A_w_o, B_w_gate, B_w_up, B_w_down, B_x, grad_out):
    _const = dict(B_x=B_x)
    def _f(*_d):
        return _fwd_reference(**{'A_x': _d[0], 'A_c_kv': _d[1], 'A_w_q': _d[2], 'A_w_uk': _d[3], 'A_w_uv': _d[4], 'A_w_o': _d[5], 'B_w_gate': _d[6], 'B_w_up': _d[7], 'B_w_down': _d[8], **_const})
    _out, _vjp = jax.vjp(_f, A_x, A_c_kv, A_w_q, A_w_uk, A_w_uv, A_w_o, B_w_gate, B_w_up, B_w_down)
    _grads = _vjp(grad_out)
    _out0 = jnp.asarray(_out)
    return (_out0, *[jnp.asarray(_g) for _g in _grads])
```

```python
import jax
import jax.numpy as jnp
from jax.experimental import pallas as pl
from jax.experimental.pallas import tpu as pltpu

BF16 = jnp.bfloat16
F32 = jnp.float32

_NT = (((1,), (1,)), ((), ()))
_TN = (((0,), (0,)), ((), ()))

_LN_EPS = 1e-5
_GELU_C = 0.7978845608028654
_GELU_A = 0.044715

_CK_REGIONS = 4
_W_REGIONS = 4
_F_REGIONS = 2
_PIECE_ROWS = 32
_DRAIN_AT = 6
_TAIL_ROWS = 400
_CK_SEM = 4


def _dot(a, b, dims=None):
    if dims is None:
        return jnp.dot(a, b, preferred_element_type=F32)
    return jax.lax.dot_general(a, b, dims, preferred_element_type=F32)


def _bmm(eq, a, b):
    return jnp.einsum(eq, a, b, preferred_element_type=F32)


def _kernel(
    x_hbm, ckv_hbm, wq_hbm, wuk_hbm, wuv_hbm, wo_hbm, wg_hbm, wu_hbm, wd_hbm, go_hbm,
    out_hbm, dx_hbm, dckv_hbm, dwq_hbm, dwuk_hbm, dwuv_hbm, dwo_hbm, dwg_hbm, dwu_hbm, dwd_hbm,
    x_v, go_v, out_v, dx_v,
    ck_v, wq_v, wuk_v, wuv_v, wo_v, wg_v, wu_v, wd_v,
    wq_t, wuk_t, wuv_t, qq_v, r_v,
    sems,
):
    nb = ck_v.shape[0]
    dc = ck_v.shape[-1]
    sk = ck_v.shape[1] * ck_v.shape[2]
    nh, dm, hd = wq_t.shape
    nf = wg_v.shape[0] * wg_v.shape[1]
    scale = float(hd) ** -0.5
    b0 = _DRAIN_AT

    head = wd_v.shape[1] - _TAIL_ROWS
    reads = {
        "wo": (wo_hbm, wo_v, 0), "x": (x_hbm, x_v, 0), "go": (go_hbm, go_v, 0),
        "wuv": (wuv_hbm, wuv_v, 1), "wq": (wq_hbm, wq_v, 2), "wuk": (wuk_hbm, wuk_v, 3),
        **{"ck%d" % b: (ckv_hbm.at[b], ck_v.at[b], _CK_SEM + b if b < b0 else 0)
           for b in range(nb)},
        "wg": (wg_hbm, wg_v, 0), "wu": (wu_hbm, wu_v, 0),
        "wd0": (wd_hbm.at[0], wd_v.at[0], 0),
        "wd1": (wd_hbm.at[1, pl.ds(0, head)], wd_v.at[1, pl.ds(0, head)], 0),
        "tail": (wd_hbm.at[1, pl.ds(head, _TAIL_ROWS)], wd_v.at[1, pl.ds(head, _TAIL_ROWS)], 1),
    }
    first_reads = ["wo", "x", "go", "wuv", "wq", "wuk"] + ["ck%d" % b for b in range(b0)]
    drain_reads = ["ck%d" % b for b in range(b0, nb)] + ["wg", "wu", "wd0", "wd1"]

    def rd(name):
        src, dst, slot = reads[name]
        return pltpu.make_async_copy(src, dst, sems.at[slot])

    def rd_ck(b):
        return pltpu.make_async_copy(ckv_hbm.at[b], ck_v.at[b], sems.at[_CK_SEM + b])

    assert sems.shape[0] >= 10
    writes = {
        "ck_lo": (ck_v.at[0:b0], dckv_hbm.at[0:b0], 4),
        "ck_hi": (ck_v.at[b0:nb], dckv_hbm.at[b0:nb], 5),
        "wo": (wo_v, dwo_hbm, 6), "wuv": (wuv_v, dwuv_hbm, 7),
        "wuk": (wuk_v, dwuk_hbm, 8), "wq": (wq_v, dwq_hbm, 9),
        "wg": (wg_v, dwg_hbm, 2), "wu": (wu_v, dwu_hbm, 3), "wd": (wd_v, dwd_hbm, 0),
    }

    def wr_pieces(name, axis, step):
        src, dst, slot = writes[name]
        n = src.shape[axis]
        copies = []
        for o in range(0, n, step):
            idx = (slice(None),) * axis + (pl.ds(o, min(step, n - o)),)
            copies.append(pltpu.make_async_copy(src.at[idx], dst.at[idx], sems.at[slot]))
        return copies

    def wr_start(name, axis, step):
        for cp in wr_pieces(name, axis, step):
            cp.start()

    def wr_start_interleaved(*specs):
        for group in zip(*[wr_pieces(name, 1, step) for name, step in specs], strict=True):
            for cp in group:
                cp.start()

    def wr_wait(name):
        src, dst, slot = writes[name]
        pltpu.make_async_copy(src, dst, sems.at[slot]).wait()

    for name in first_reads:
        rd(name).start()

    def to_head_major(src, dst):
        nr, nc = src.shape[0], src.shape[1]
        for r in range(nr):
            dst[:, pl.ds(r * nc, nc), :] = jnp.swapaxes(src[r], 0, 1)

    for name in ("wo", "x", "go"):
        rd(name).wait()
    for name in drain_reads:
        rd(name).start()
    x = x_v[...].astype(F32)
    go = go_v[...].astype(F32)
    xc = x - jnp.mean(x, axis=-1, keepdims=True)
    rstd = jax.lax.rsqrt(jnp.mean(xc * xc, axis=-1, keepdims=True) + _LN_EPS)
    xn = xc * rstd
    xn_b = xn.astype(BF16)
    go_b = go.astype(BF16)
    xn_h = jnp.broadcast_to(xn_b[None], (nh,) + xn_b.shape)
    go_h = jnp.broadcast_to(go_b[None], (nh,) + go_b.shape)

    def wo3():
        return wo_v[...].reshape(nh, hd, dm)

    d_ctx = _bmm("hbm,hdm->hbd", go_h, wo3()).astype(BF16)
    rd("wuv").wait()
    rd("tail").start()
    to_head_major(wuv_v, wuv_t)
    d_cc = _bmm("hbd,hcd->hbc", d_ctx, wuv_t[...])
    rd("wq").wait()
    to_head_major(wq_v, wq_t)
    q = _bmm("hbm,hmd->hbd", xn_h, wq_t[...]).astype(BF16)
    rd("wuk").wait()
    to_head_major(wuk_v, wuk_t)
    qs = _bmm("hbd,hcd->hbc", q, wuk_t[...]) * scale
    qq_v[...] = jnp.swapaxes(jnp.concatenate([qs, d_cc], axis=0), 0, 1).astype(BF16)

    def attend(b):
        qq = qq_v[b]
        s_all = _dot(qq, ck_v[b].reshape(sk, dc), _NT)
        s = s_all[:nh]
        dp = s_all[nh:]
        e = jnp.exp(s - jnp.max(s, axis=1, keepdims=True))
        p = e * (1.0 / jnp.sum(e, axis=1, keepdims=True))
        ds = p * (dp - jnp.sum(p * dp, axis=1, keepdims=True))
        pp = jnp.concatenate([ds, p], axis=0).astype(BF16)
        r_v[b] = _dot(pp, ck_v[b].reshape(sk, dc))
        ck_v[b] = _dot(pp, qq, _TN).astype(BF16).reshape(ck_v.shape[1:])

    def early_rows(b, carry):
        rd_ck(b).wait()
        attend(b)
        return carry

    jax.lax.fori_loop(0, b0, early_rows, 0)

    for name in drain_reads:
        rd(name).wait()
    wr_start("ck_lo", 2, _PIECE_ROWS)
    rd("tail").wait()

    def late_rows(b, carry):
        attend(b)
        return carry

    jax.lax.fori_loop(b0, nb, late_rows, 0)
    wr_start("ck_hi", 2, _PIECE_ROWS)

    r = jnp.swapaxes(r_v[...], 0, 1)
    d_qa = (r[:nh] * scale).astype(BF16)
    cc = r[nh:].astype(BF16)
    ctx = _bmm("hbc,hcd->hbd", cc, wuv_t[...]).astype(BF16)
    d_q = _bmm("hbc,hcd->hbd", d_qa, wuk_t[...]).astype(BF16)
    attn_out = jnp.sum(_bmm("hbd,hdm->hbm", ctx, wo3()), axis=0)
    d_xn = jnp.sum(_bmm("hbd,hmd->hbm", d_q, wq_t[...]), axis=0)

    def head_grad(a, bmat, dst):
        nr, nc = dst.shape[0], dst.shape[1]
        for r in range(nr):
            g = _bmm("hbc,hbd->hcd", a[:, :, r * nc:(r + 1) * nc], bmat).astype(BF16)
            dst[r] = jnp.swapaxes(g, 0, 1)

    m_step = (_PIECE_ROWS * dm) // (nh * hd)
    wo_v[...] = _bmm("hbd,hbm->hdm", ctx, go_h).astype(BF16).reshape(wo_v.shape)
    head_grad(cc, d_ctx, wuv_v)
    wr_start_interleaved(("wo", _PIECE_ROWS), ("wuv", m_step))
    head_grad(d_qa, q, wuk_v)
    head_grad(xn_h, d_q, wq_v)
    wr_start_interleaved(("wuk", m_step), ("wq", m_step))

    wg = wg_v[...].reshape(nf, dm)
    wu = wu_v[...].reshape(nf, dm)
    wd = wd_v[...].reshape(nf, dm)
    g = _dot(xn_b, wg, _NT)
    u = _dot(xn_b, wu, _NT)
    t = jnp.tanh(_GELU_C * (g + _GELU_A * g * g * g))
    gel = 0.5 * g * (1.0 + t)
    dgel = 0.5 * (1.0 + t) + 0.5 * g * (1.0 - t * t) * _GELU_C * (1.0 + 3.0 * _GELU_A * g * g)
    hh = (gel * u).astype(BF16)
    ffn = _dot(hh, wd)
    d_hh = _dot(go_b, wd, _NT)
    d_g = (d_hh * u * dgel).astype(BF16)
    d_u = (d_hh * gel).astype(BF16)
    d_xn = d_xn + _dot(d_g, wg) + _dot(d_u, wu)

    out_v[...] = (x + attn_out + ffn).astype(BF16)
    dx = go + rstd * (d_xn - jnp.mean(d_xn, axis=-1, keepdims=True)
                      - xn * jnp.mean(d_xn * xn, axis=-1, keepdims=True))
    dx_v[...] = dx.astype(BF16)
    small = [pltpu.make_async_copy(out_v, out_hbm, sems.at[1]),
             pltpu.make_async_copy(dx_v, dx_hbm, sems.at[1])]
    for cp in small:
        cp.start()

    wg_v[...] = _dot(d_g, xn_b, _TN).astype(BF16).reshape(wg_v.shape)
    wu_v[...] = _dot(d_u, xn_b, _TN).astype(BF16).reshape(wu_v.shape)
    wd_v[...] = _dot(hh, go_b, _TN).astype(BF16).reshape(wd_v.shape)
    wr_start_interleaved(*[(k, _PIECE_ROWS) for k in ("wg", "wu", "wd")])

    for cp in small:
        cp.wait()
    for name in writes:
        wr_wait(name)


@jax.jit
def pallas_parallel_sum__compressed_kv_cla__geglu_ffn__decode_kernel(
    A_x, A_c_kv, A_w_q, A_w_uk, A_w_uv, A_w_o, B_x, B_w_gate, B_w_up, B_w_down, grad_out,
):
    del B_x
    nb, sk, dc = A_c_kv.shape
    dm, nh, hd = A_w_q.shape
    nf = B_w_down.shape[0]
    ins = (
        A_x.reshape(nb, dm),
        A_c_kv.reshape(nb, _CK_REGIONS, sk // _CK_REGIONS, dc),
        A_w_q.reshape(_W_REGIONS, dm // _W_REGIONS, nh, hd),
        A_w_uk.reshape(_W_REGIONS, dc // _W_REGIONS, nh, hd),
        A_w_uv.reshape(_W_REGIONS, dc // _W_REGIONS, nh, hd),
        A_w_o.reshape(_W_REGIONS, nh * hd // _W_REGIONS, dm),
        B_w_gate.T.reshape(_F_REGIONS, nf // _F_REGIONS, dm),
        B_w_up.T.reshape(_F_REGIONS, nf // _F_REGIONS, dm),
        B_w_down.reshape(_F_REGIONS, nf // _F_REGIONS, dm),
        grad_out.reshape(nb, dm),
    )
    x2, ck4, wq4, wuk4, wuv4, wo3, wg3, wu3, wd3, _ = ins
    like = lambda a: jax.ShapeDtypeStruct(a.shape, a.dtype)
    out_shape = tuple(like(a) for a in (x2, x2, ck4, wq4, wuk4, wuv4, wo3, wg3, wu3, wd3))
    vmem = lambda shape, dtype=BF16: pltpu.VMEM(tuple(shape), dtype)
    scratch = [
        vmem(x2.shape), vmem(x2.shape), vmem(x2.shape), vmem(x2.shape),
        vmem(ck4.shape), vmem(wq4.shape), vmem(wuk4.shape), vmem(wuv4.shape), vmem(wo3.shape),
        vmem(wg3.shape), vmem(wu3.shape), vmem(wd3.shape),
        vmem((nh, dm, hd)), vmem((nh, dc, hd)), vmem((nh, dc, hd)),
        vmem((nb, 2 * nh, dc)), vmem((nb, 2 * nh, dc), F32),
        pltpu.SemaphoreType.DMA((_CK_SEM + _DRAIN_AT,)),
    ]
    hbm = pl.BlockSpec(memory_space=pltpu.HBM)
    out, dx, dckv, dwq, dwuk, dwuv, dwo, dwg_t, dwu_t, dwd = pl.pallas_call(
        _kernel,
        out_shape=out_shape,
        in_specs=[hbm] * len(ins),
        out_specs=tuple([hbm] * len(out_shape)),
        scratch_shapes=scratch,
        compiler_params=pltpu.CompilerParams(vmem_limit_bytes=100 * 1024 * 1024),
    )(*ins)
    return (
        out.reshape(A_x.shape), dx.reshape(A_x.shape), dckv.reshape(A_c_kv.shape),
        dwq.reshape(A_w_q.shape), dwuk.reshape(A_w_uk.shape), dwuv.reshape(A_w_uv.shape),
        dwo.reshape(A_w_o.shape),
        dwg_t.reshape(nf, dm).T, dwu_t.reshape(nf, dm).T, dwd.reshape(nf, dm),
    )
```
